```python
import os as _os
_os.environ.setdefault("JAX_PLATFORMS", "cpu")
import jax
import jax.numpy as jnp

def _softmax(x, axis=-1):
    return jax.nn.softmax(x, axis=axis)
def _gelu(x):
    return jax.nn.gelu(x, approximate=True)
def _silu(x):
    return jax.nn.silu(x)
def _sigmoid(x):
    return jax.nn.sigmoid(x)
def _layernorm(x, axis=-1, eps=1e-5):
    m = jnp.mean(x, axis=axis, keepdims=True)
    v = jnp.var(x, axis=axis, keepdims=True)
    return (x - m) / jnp.sqrt(v + eps)
def _scatter_add(tgt, idx, src, axis=0):
    return tgt.at[idx].add(src)
def _segment_sum(src, seg, n):
    return jax.ops.segment_sum(src, seg, n)
class _Rng:
    def __init__(self, key):
        self._k = key
    def _next(self):
        self._k, sub = jax.random.split(self._k)
        return sub
    def normal(self, shape):
        return jax.random.normal(self._next(), shape, dtype=jnp.bfloat16)
    def randint(self, lo, hi, shape):
        return jax.random.randint(self._next(), shape, lo, hi, dtype=jnp.int32)
    def uniform(self, shape, lo=0.0, hi=1.0):
        return jax.random.uniform(self._next(), shape, jnp.bfloat16, lo, hi)
    def permutation(self, n):
        return jax.random.permutation(self._next(), n)


kernel_name = 'sequential_preLN__mha_block__dense_activation_mish__prompt'

def setup_inputs():
    _rng = _Rng(jax.random.key(int.from_bytes(__import__("os").urandom(4), "little")))
    _w = (lambda a: (lambda t: t.astype(jnp.bfloat16) if jnp.issubdtype(t.dtype, jnp.floating) else t)(jnp.asarray(a)))
    def _A_setup():
        B, S, D, H = 1, 2048, 576, 32
        return {
            "x": _w((lambda *s: _rng.normal(s) * 0.05)(B, S, D)),
            "wqkv": _w((lambda *s: _rng.normal(s) * 0.05)(D, 3 * D)),
            "wo": _w((lambda *s: _rng.normal(s) * 0.05)(D, D)),
        }
    _A_in = _A_setup()

    def _B_setup():
        B, S, D, F = 1, 2048, 576, 4608
        return {
            "x": _w((lambda *s: _rng.normal(s) * 0.05)(B, S, D)),
            "w1": _w((lambda *s: _rng.normal(s) * 1.6)(D, F) * (D ** -0.5)),
            "b1": _w((lambda *s: _rng.normal(s) * 0.05)(F)),
            "w2": _w((lambda *s: _rng.normal(s) * 0.05)(F, D) * (F ** -0.5)),
        }
    _B_in = _B_setup()

    return {
        "A_x": _A_in["x"],
        "A_wqkv": _A_in["wqkv"],
        "A_wo": _A_in["wo"],
        "B_x": _B_in["x"],
        "B_w1": _B_in["w1"],
        "B_b1": _B_in["b1"],
        "B_w2": _B_in["w2"],
    }

def reference(A_x, A_wqkv, A_wo, B_x, B_w1, B_b1, B_w2):
    def _A_ref(x, wqkv, wo):
        B, S, D = x.shape
        H = 32
        Dh = D // H
        qkv = (lambda x, *d: x.transpose(*d))((x @ wqkv).reshape(B, S, 3, H, Dh), 2, 0, 3, 1, 4)
        q, k, v = qkv[0], qkv[1], qkv[2]
        scores = jnp.einsum("bhqd,bhkd->bhqk", q, k) * (Dh ** -0.5)
        p = _softmax(scores, axis=-1)
        o = jnp.einsum("bhqk,bhkd->bhqd", p, v)
        return (lambda x, *d: x.transpose(*d))(o, 0, 2, 1, 3).reshape(B, S, D) @ wo

    def _B_ref(x, w1, b1, w2):
        h = jnp.einsum("bsd,df->bsf", x, w1) + b1
        sp = jnp.log1p(jnp.exp(-jnp.abs(h))) + jnp.where(h > 0, h, jnp.zeros_like(h))
        act = h * jnp.tanh(sp)
        return jnp.einsum("bsf,fd->bsd", act, w2)

    x = A_x
    h = x + _A_ref(_layernorm(x, axis=-1), A_wqkv, A_wo)
    h2 = h + _B_ref(_layernorm(h, axis=-1), B_w1, B_b1, B_w2)
    return h2
```

```python
import functools
import math

import jax
import jax.numpy as jnp
import jax.experimental.pallas as pl
import jax.experimental.pallas.tpu as pltpu

S = 2048
D = 576
H = 32
DH = 18
F = 4608
HPG = 7
NG = 5
GW = 128
DP = NG * GW
SUM_LANE = HPG * DH
EPS = 1e-5

TQ = 256
PROJ_CHUNK = 256
FC = 1536


def _layernorm(x):
    m = jnp.mean(x, axis=-1, keepdims=True)
    xc = x - m
    v = jnp.mean(xc * xc, axis=-1, keepdims=True)
    return xc * jax.lax.rsqrt(v + EPS)


def _kernel(x_ref, wqkv_ref, wo_ref, w1_ref, b1_ref, w2_ref, o_ref,
            q_sc, k_sc, v_sc):
    step = pl.program_id(0)
    q_scale = (DH ** -0.5) * math.log2(math.e)

    @pl.when(step == 0)
    def _():
        lane = jax.lax.broadcasted_iota(jnp.int32, (PROJ_CHUNK, GW), 1)

        def proj(c, carry):
            r0 = pl.multiple_of(c * PROJ_CHUNK, PROJ_CHUNK)
            xr = x_ref[pl.ds(r0, PROJ_CHUNK), :].astype(jnp.float32)
            xn = _layernorm(xr).astype(jnp.bfloat16)
            qkv = jnp.dot(xn, wqkv_ref[...], preferred_element_type=jnp.float32)
            for g in range(NG):
                q_sc[g, pl.ds(r0, PROJ_CHUNK), :] = (
                    qkv[:, g * GW:(g + 1) * GW] * q_scale).astype(jnp.bfloat16)
                k_sc[g, pl.ds(r0, PROJ_CHUNK), :] = (
                    qkv[:, DP + g * GW:DP + (g + 1) * GW]).astype(jnp.bfloat16)
                vg = qkv[:, 2 * DP + g * GW:2 * DP + (g + 1) * GW]
                vg = jnp.where(lane == SUM_LANE, 1.0, vg)
                v_sc[g, pl.ds(r0, PROJ_CHUNK), :] = vg.astype(jnp.bfloat16)
            return carry

        jax.lax.fori_loop(0, S // PROJ_CHUNK, proj, 0)

    q0 = pl.multiple_of(step * TQ, TQ)
    lane = jax.lax.broadcasted_iota(jnp.int32, (TQ, GW), 1)
    o_groups = []
    for g in range(NG):
        qg = q_sc[g, pl.ds(q0, TQ), :]
        kg = k_sc[g]
        vg = v_sc[g]
        n_heads = min(HPG, H - g * HPG)

        def head(j, og, qg=qg, kg=kg, vg=vg):
            sel = jnp.logical_and(lane >= j * DH, lane < (j + 1) * DH)
            qm = jnp.where(sel, qg, jnp.zeros_like(qg))
            s = jax.lax.dot_general(qm, kg, (((1,), (1,)), ((), ())),
                                    preferred_element_type=jnp.float32)
            m = jnp.max(s, axis=-1, keepdims=True)
            p = jnp.exp2(s - m).astype(jnp.bfloat16)
            of = jnp.dot(p, vg, preferred_element_type=jnp.float32)
            l = of[:, SUM_LANE:SUM_LANE + 1]
            return jnp.where(sel, of / l, og)

        og = jax.lax.fori_loop(0, n_heads, head,
                               jnp.zeros((TQ, GW), jnp.float32))
        o_groups.append(og.astype(jnp.bfloat16))
    o_all = jnp.concatenate(o_groups, axis=-1)
    attn = jnp.dot(o_all, wo_ref[...], preferred_element_type=jnp.float32)
    h = x_ref[pl.ds(q0, TQ), :].astype(jnp.float32) + attn

    hn = _layernorm(h).astype(jnp.bfloat16)
    acc = h
    for c in range(F // FC):
        a = jnp.dot(hn, w1_ref[:, c * FC:(c + 1) * FC],
                    preferred_element_type=jnp.float32)
        a = a + b1_ref[:, c * FC:(c + 1) * FC].astype(jnp.float32)
        sp = jnp.log1p(jnp.exp(-jnp.abs(a))) + jnp.maximum(a, 0.0)
        act = (a * jnp.tanh(sp)).astype(jnp.bfloat16)
        acc = acc + jnp.dot(act, w2_ref[c * FC:(c + 1) * FC, :],
                            preferred_element_type=jnp.float32)
    o_ref[...] = acc.astype(o_ref.dtype)


def _pad_heads_cols(w):
    w = w.reshape(D, H, DH)
    w = jnp.pad(w, ((0, 0), (0, NG * HPG - H), (0, 0)))
    w = w.reshape(D, NG, HPG * DH)
    w = jnp.pad(w, ((0, 0), (0, 0), (0, GW - HPG * DH)))
    return w.reshape(D, DP)


@jax.jit
def pallas_sequential_preLN__mha_block__dense_activation_mish__prompt_kernel(
    A_x: jax.Array,
    A_wqkv: jax.Array,
    A_wo: jax.Array,
    B_x: jax.Array,
    B_w1: jax.Array,
    B_b1: jax.Array,
    B_w2: jax.Array,
):
    x = A_x.reshape(S, D)
    wqkv = jnp.concatenate(
        [_pad_heads_cols(A_wqkv[:, i * D:(i + 1) * D]) for i in range(3)], axis=1)
    wo = A_wo.reshape(H, DH, D)
    wo = jnp.pad(wo, ((0, NG * HPG - H), (0, 0), (0, 0)))
    wo = wo.reshape(NG, HPG * DH, D)
    wo = jnp.pad(wo, ((0, 0), (0, GW - HPG * DH), (0, 0))).reshape(DP, D)
    b1 = B_b1.reshape(1, F)

    const = lambda i: (0, 0)
    out = pl.pallas_call(
        _kernel,
        grid=(S // TQ,),
        in_specs=[
            pl.BlockSpec((S, D), const),
            pl.BlockSpec((D, 3 * DP), const),
            pl.BlockSpec((DP, D), const),
            pl.BlockSpec((D, F), const),
            pl.BlockSpec((1, F), const),
            pl.BlockSpec((F, D), const),
        ],
        out_specs=pl.BlockSpec((TQ, D), lambda i: (i, 0)),
        out_shape=jax.ShapeDtypeStruct((S, D), A_x.dtype),
        scratch_shapes=[
            pltpu.VMEM((NG, S, GW), jnp.bfloat16),
            pltpu.VMEM((NG, S, GW), jnp.bfloat16),
            pltpu.VMEM((NG, S, GW), jnp.bfloat16),
        ],
        compiler_params=pltpu.CompilerParams(
            dimension_semantics=("arbitrary",),
            vmem_limit_bytes=100 * 1024 * 1024,
        ),
    )(x, wqkv, wo, B_w1, b1, B_w2)
    return out.reshape(A_x.shape)
```

```python
import math

import jax
import jax.numpy as jnp
import jax.experimental.pallas as pl
import jax.experimental.pallas.tpu as pltpu

S = 2048
D = 576
H = 32
DH = 18
F = 4608
HPG = 7
NG = 5
GW = 128
DP = NG * GW
VR = 32
OR = 24
EPS = 1e-5

TQ = 256
PROJ_CHUNK = 256
FC = 1536


def _layernorm(x):
    m = jnp.mean(x, axis=-1, keepdims=True)
    xc = x - m
    v = jnp.mean(xc * xc, axis=-1, keepdims=True)
    return xc * jax.lax.rsqrt(v + EPS)


def _kernel(x_ref, wqkv_ref, wo_ref, w1_hbm, b1_ref, w2_hbm, o_ref,
            wp_sc, wo_sc, q_sc, k_sc, vt_sc, ot_sc, sa_sc, sb_sc,
            w1_ref, w2_ref, sems):
    step = pl.program_id(0)
    q_scale = (DH ** -0.5) * math.log2(math.e)
    w1_copy = pltpu.make_async_copy(w1_hbm, w1_ref, sems.at[0])
    w2_copy = pltpu.make_async_copy(w2_hbm, w2_ref, sems.at[1])

    @pl.when(step == 0)
    def _():
        w1_copy.start()
        w2_copy.start()
        w = wqkv_ref[...].astype(jnp.float32)
        pieces = []
        for t in range(2):
            for g in range(NG):
                lo = g * HPG * DH
                hi = min(lo + HPG * DH, D)
                pieces.append(w[:, t * D + lo:t * D + hi])
                pieces.append(jnp.zeros((D, GW - (hi - lo)), jnp.float32))
        for hh in range(H):
            pieces.append(w[:, 2 * D + hh * DH:2 * D + (hh + 1) * DH])
            pieces.append(jnp.zeros((D, VR - DH), jnp.float32))
        wp_sc[...] = jnp.concatenate(pieces, axis=1).astype(jnp.bfloat16)
        wo = wo_ref[...].astype(jnp.float32)
        rows = []
        for hh in range(H):
            rows.append(wo[hh * DH:(hh + 1) * DH, :])
            rows.append(jnp.zeros((OR - DH, D), jnp.float32))
        wo_sc[...] = jnp.concatenate(rows, axis=0).astype(jnp.bfloat16)

        vrow = jax.lax.broadcasted_iota(jnp.int32, (H * VR, PROJ_CHUNK), 0)
        ones_row = (vrow % VR) == DH

        def proj(c, carry):
            r0 = pl.multiple_of(c * PROJ_CHUNK, PROJ_CHUNK)
            xr = x_ref[:, pl.ds(r0, PROJ_CHUNK)].astype(jnp.float32).T
            xn = _layernorm(xr).astype(jnp.bfloat16)
            qkv = jnp.dot(xn, wp_sc[...], preferred_element_type=jnp.float32)
            for g in range(NG):
                q_sc[g, pl.ds(r0, PROJ_CHUNK), :] = (
                    qkv[:, g * GW:(g + 1) * GW] * q_scale).astype(jnp.bfloat16)
                k_sc[g, pl.ds(r0, PROJ_CHUNK), :] = (
                    qkv[:, DP + g * GW:DP + (g + 1) * GW]).astype(jnp.bfloat16)
            vt = qkv[:, 2 * DP:].T
            vt = jnp.where(ones_row, 1.0, vt)
            vt_sc[:, pl.ds(r0, PROJ_CHUNK)] = vt.astype(jnp.bfloat16)
            return carry

        jax.lax.fori_loop(0, S // PROJ_CHUNK, proj, 0)

    q0 = pl.multiple_of(step * TQ, TQ)
    lane = jax.lax.broadcasted_iota(jnp.int32, (TQ, GW), 1)

    def scores(hh, s_ref):
        g = hh // HPG
        j = hh - g * HPG
        qg = q_sc[g, pl.ds(q0, TQ), :]
        sel = jnp.logical_and(lane >= j * DH, lane < (j + 1) * DH)
        qm = jnp.where(sel, qg, jnp.zeros_like(qg))
        st = jax.lax.dot_general(k_sc[g], qm, (((1,), (1,)), ((), ())),
                                 preferred_element_type=jnp.float32)
        s_ref[...] = st
        return jnp.max(st, axis=0, keepdims=True)

    def finish(hh, s_ref, m):
        pt = jnp.exp2(s_ref[...] - m).astype(jnp.bfloat16)
        vt = vt_sc[pl.ds(pl.multiple_of(hh * VR, VR), VR), :]
        ot = jnp.dot(vt, pt, preferred_element_type=jnp.float32)
        ot = ot[0:OR, :] / ot[DH:DH + 1, :]
        ot_sc[pl.ds(pl.multiple_of(hh * OR, 8), OR), :] = ot

    def head_pair(i, ma):
        hh = 2 * i
        mb = scores(hh + 1, sb_sc)
        finish(hh, sa_sc, ma)
        ma = scores(hh + 2, sa_sc)
        finish(hh + 1, sb_sc, mb)
        return ma

    ma = jax.lax.fori_loop(0, H // 2 - 1, head_pair, scores(0, sa_sc))
    mb = scores(H - 1, sb_sc)
    finish(H - 2, sa_sc, ma)
    finish(H - 1, sb_sc, mb)
    o_all = ot_sc[...].T.astype(jnp.bfloat16)
    attn = jnp.dot(o_all, wo_sc[...], preferred_element_type=jnp.float32)
    h = x_ref[:, pl.ds(q0, TQ)].astype(jnp.float32).T + attn

    @pl.when(step == 0)
    def _():
        w1_copy.wait()
        w2_copy.wait()

    hn = _layernorm(h).astype(jnp.bfloat16)
    acc = h
    for c in range(F // FC):
        a = jnp.dot(hn, w1_ref[:, c * FC:(c + 1) * FC],
                    preferred_element_type=jnp.float32)
        a = a + b1_ref[:, c * FC:(c + 1) * FC].astype(jnp.float32)
        sp = jnp.log1p(jnp.exp(-jnp.abs(a))) + jnp.maximum(a, 0.0)
        act = (a * jnp.tanh(sp)).astype(jnp.bfloat16)
        acc = acc + jax.lax.dot_general(
            act, w2_ref[:, c * FC:(c + 1) * FC], (((1,), (1,)), ((), ())),
            preferred_element_type=jnp.float32)
    o_ref[...] = acc.T.astype(o_ref.dtype)


@jax.jit
def pallas_sequential_preLN__mha_block__dense_activation_mish__prompt_kernel(
    A_x: jax.Array,
    A_wqkv: jax.Array,
    A_wo: jax.Array,
    B_x: jax.Array,
    B_w1: jax.Array,
    B_b1: jax.Array,
    B_w2: jax.Array,
):
    x = A_x.reshape(S, D).T
    b1 = B_b1.reshape(1, F)

    const = lambda i: (0, 0)
    out = pl.pallas_call(
        _kernel,
        grid=(S // TQ,),
        in_specs=[
            pl.BlockSpec((D, S), const),
            pl.BlockSpec((D, 3 * D), const),
            pl.BlockSpec((D, D), const),
            pl.BlockSpec(memory_space=pl.ANY),
            pl.BlockSpec((1, F), const),
            pl.BlockSpec(memory_space=pl.ANY),
        ],
        out_specs=pl.BlockSpec((D, TQ), lambda i: (0, i)),
        out_shape=jax.ShapeDtypeStruct((D, S), A_x.dtype),
        scratch_shapes=[
            pltpu.VMEM((D, 2 * DP + H * VR), jnp.bfloat16),
            pltpu.VMEM((H * OR, D), jnp.bfloat16),
            pltpu.VMEM((NG, S, GW), jnp.bfloat16),
            pltpu.VMEM((NG, S, GW), jnp.bfloat16),
            pltpu.VMEM((H * VR, S), jnp.bfloat16),
            pltpu.VMEM((H * OR, TQ), jnp.float32),
            pltpu.VMEM((S, TQ), jnp.float32),
            pltpu.VMEM((S, TQ), jnp.float32),
            pltpu.VMEM((D, F), jnp.bfloat16),
            pltpu.VMEM((D, F), jnp.bfloat16),
            pltpu.SemaphoreType.DMA((2,)),
        ],
        compiler_params=pltpu.CompilerParams(
            dimension_semantics=("arbitrary",),
            vmem_limit_bytes=100 * 1024 * 1024,
        ),
    )(x, A_wqkv, A_wo, B_w1, b1, B_w2.T)
    return out.T.reshape(A_x.shape)
```

```python
import math

import jax
import jax.numpy as jnp
import jax.experimental.pallas as pl
import jax.experimental.pallas.tpu as pltpu

S = 2048
D = 576
H = 32
DH = 18
F = 4608
HPG = 7
NG = 5
GW = 128
DP = NG * GW
VR = 32
OR = 24
EPS = 1e-5

TQ = 256
PROJ_CHUNK = 256
FC = 1536


def _layernorm(x):
    m = jnp.mean(x, axis=-1, keepdims=True)
    xc = x - m
    v = jnp.mean(xc * xc, axis=-1, keepdims=True)
    return xc * jax.lax.rsqrt(v + EPS)


def _kernel(x_ref, wqkv_ref, wo_ref, w1_hbm, b1_ref, w2_hbm, o_ref,
            wp_sc, wo_sc, q_sc, k_sc, vt_sc, ot_sc, sa_sc, sb_sc,
            w1_ref, w2_ref, sems):
    step = pl.program_id(0)
    q_scale = (DH ** -0.5) * math.log2(math.e)
    w1_copy = pltpu.make_async_copy(w1_hbm, w1_ref, sems.at[0])
    w2_copy = pltpu.make_async_copy(w2_hbm, w2_ref, sems.at[1])

    @pl.when(step == 0)
    def _():
        w1_copy.start()
        w2_copy.start()
        w = wqkv_ref[...].astype(jnp.float32)
        pieces = []
        for t in range(2):
            for g in range(NG):
                lo = g * HPG * DH
                hi = min(lo + HPG * DH, D)
                pieces.append(w[:, t * D + lo:t * D + hi])
                pieces.append(jnp.zeros((D, GW - (hi - lo)), jnp.float32))
        for hh in range(H):
            pieces.append(w[:, 2 * D + hh * DH:2 * D + (hh + 1) * DH])
            pieces.append(jnp.zeros((D, VR - DH), jnp.float32))
        wp_sc[...] = jnp.concatenate(pieces, axis=1).astype(jnp.bfloat16)
        wo = wo_ref[...].astype(jnp.float32)
        rows = []
        for hh in range(H):
            rows.append(wo[hh * DH:(hh + 1) * DH, :])
            rows.append(jnp.zeros((OR - DH, D), jnp.float32))
        wo_sc[...] = jnp.concatenate(rows, axis=0).astype(jnp.bfloat16)

        vrow = jax.lax.broadcasted_iota(jnp.int32, (H * VR, PROJ_CHUNK), 0)
        ones_row = (vrow % VR) == DH

        def proj(c, carry):
            r0 = pl.multiple_of(c * PROJ_CHUNK, PROJ_CHUNK)
            xr = x_ref[:, pl.ds(r0, PROJ_CHUNK)].astype(jnp.float32).T
            xn = _layernorm(xr).astype(jnp.bfloat16)
            qkv = jnp.dot(xn, wp_sc[...], preferred_element_type=jnp.float32)
            for g in range(NG):
                q_sc[g, pl.ds(r0, PROJ_CHUNK), :] = (
                    qkv[:, g * GW:(g + 1) * GW] * q_scale).astype(jnp.bfloat16)
                k_sc[g, pl.ds(r0, PROJ_CHUNK), :] = (
                    qkv[:, DP + g * GW:DP + (g + 1) * GW]).astype(jnp.bfloat16)
            vt = qkv[:, 2 * DP:].T
            vt = jnp.where(ones_row, 1.0, vt)
            vt_sc[:, pl.ds(r0, PROJ_CHUNK)] = vt.astype(jnp.bfloat16)
            return carry

        jax.lax.fori_loop(0, S // PROJ_CHUNK, proj, 0)

    q0 = pl.multiple_of(step * TQ, TQ)
    lane = jax.lax.broadcasted_iota(jnp.int32, (TQ, GW), 1)

    def scores(hh, s_ref):
        g = hh // HPG
        j = hh - g * HPG
        qg = q_sc[g, pl.ds(q0, TQ), :]
        sel = jnp.logical_and(lane >= j * DH, lane < (j + 1) * DH)
        qm = jnp.where(sel, qg, jnp.zeros_like(qg))
        st = jax.lax.dot_general(k_sc[g], qm, (((1,), (1,)), ((), ())),
                                 preferred_element_type=jnp.float32)
        s_ref[...] = st
        return jnp.max(st, axis=0, keepdims=True)

    def finish(hh, s_ref, m):
        pt = jnp.exp2(s_ref[...] - m).astype(jnp.bfloat16)
        vt = vt_sc[pl.ds(pl.multiple_of(hh * VR, VR), VR), :]
        ot = jnp.dot(vt, pt, preferred_element_type=jnp.float32)
        ot = ot[0:OR, :] / ot[DH:DH + 1, :]
        ot_sc[pl.ds(pl.multiple_of(hh * OR, 8), OR), :] = ot

    def stage(hh, m, cur_ref, nxt_ref):
        m_next = scores(hh + 1, nxt_ref)
        finish(hh, cur_ref, m)
        return m_next

    def head(hh, m):
        return jax.lax.cond(hh % 2 == 0,
                            lambda m: stage(hh, m, sa_sc, sb_sc),
                            lambda m: stage(hh, m, sb_sc, sa_sc), m)

    m_last = jax.lax.fori_loop(0, H - 1, head, scores(0, sa_sc))
    finish(H - 1, sb_sc, m_last)
    o_all = ot_sc[...].T.astype(jnp.bfloat16)
    attn = jnp.dot(o_all, wo_sc[...], preferred_element_type=jnp.float32)
    h = x_ref[:, pl.ds(q0, TQ)].astype(jnp.float32).T + attn

    @pl.when(step == 0)
    def _():
        w1_copy.wait()
        w2_copy.wait()

    hn = _layernorm(h).astype(jnp.bfloat16)
    acc = h
    for c in range(F // FC):
        a = jnp.dot(hn, w1_ref[:, c * FC:(c + 1) * FC],
                    preferred_element_type=jnp.float32)
        a = a + b1_ref[:, c * FC:(c + 1) * FC].astype(jnp.float32)
        sp = jnp.log1p(jnp.exp(-jnp.abs(a))) + jnp.maximum(a, 0.0)
        act = (a * jnp.tanh(sp)).astype(jnp.bfloat16)
        acc = acc + jax.lax.dot_general(
            act, w2_ref[:, c * FC:(c + 1) * FC], (((1,), (1,)), ((), ())),
            preferred_element_type=jnp.float32)
    o_ref[...] = acc.T.astype(o_ref.dtype)


@jax.jit
def pallas_sequential_preLN__mha_block__dense_activation_mish__prompt_kernel(
    A_x: jax.Array,
    A_wqkv: jax.Array,
    A_wo: jax.Array,
    B_x: jax.Array,
    B_w1: jax.Array,
    B_b1: jax.Array,
    B_w2: jax.Array,
):
    x = A_x.reshape(S, D).T
    b1 = B_b1.reshape(1, F)

    const = lambda i: (0, 0)
    out = pl.pallas_call(
        _kernel,
        grid=(S // TQ,),
        in_specs=[
            pl.BlockSpec((D, S), const),
            pl.BlockSpec((D, 3 * D), const),
            pl.BlockSpec((D, D), const),
            pl.BlockSpec(memory_space=pl.ANY),
            pl.BlockSpec((1, F), const),
            pl.BlockSpec(memory_space=pl.ANY),
        ],
        out_specs=pl.BlockSpec((D, TQ), lambda i: (0, i)),
        out_shape=jax.ShapeDtypeStruct((D, S), A_x.dtype),
        scratch_shapes=[
            pltpu.VMEM((D, 2 * DP + H * VR), jnp.bfloat16),
            pltpu.VMEM((H * OR, D), jnp.bfloat16),
            pltpu.VMEM((NG, S, GW), jnp.bfloat16),
            pltpu.VMEM((NG, S, GW), jnp.bfloat16),
            pltpu.VMEM((H * VR, S), jnp.bfloat16),
            pltpu.VMEM((H * OR, TQ), jnp.float32),
            pltpu.VMEM((S, TQ), jnp.float32),
            pltpu.VMEM((S, TQ), jnp.float32),
            pltpu.VMEM((D, F), jnp.bfloat16),
            pltpu.VMEM((D, F), jnp.bfloat16),
            pltpu.SemaphoreType.DMA((2,)),
        ],
        compiler_params=pltpu.CompilerParams(
            dimension_semantics=("arbitrary",),
            vmem_limit_bytes=100 * 1024 * 1024,
        ),
    )(x, A_wqkv, A_wo, B_w1, b1, B_w2.T)
    return out.T.reshape(A_x.shape)
```
